```python
import jax
import jax.numpy as jnp

def _softmax(x, axis=-1):
    return jax.nn.softmax(x, axis=axis)
def _gelu(x):
    return jax.nn.gelu(x, approximate=True)
def _silu(x):
    return jax.nn.silu(x)
def _sigmoid(x):
    return jax.nn.sigmoid(x)
def _layernorm(x, axis=-1, eps=1e-5):
    m = jnp.mean(x, axis=axis, keepdims=True)
    v = jnp.var(x, axis=axis, keepdims=True)
    return (x - m) / jnp.sqrt(v + eps)
def _scatter_add(tgt, idx, src, axis=0):
    return tgt.at[idx].add(src)
def _segment_sum(src, seg, n):
    return jax.ops.segment_sum(src, seg, n)
class _Rng:
    def __init__(self, key):
        self._k = key
    def _next(self):
        self._k, sub = jax.random.split(self._k)
        return sub
    def normal(self, shape):
        return jax.random.normal(self._next(), shape, dtype=jnp.bfloat16)
    def randint(self, lo, hi, shape):
        return jax.random.randint(self._next(), shape, lo, hi, dtype=jnp.int32)
    def uniform(self, shape, lo=0.0, hi=1.0):
        return jax.random.uniform(self._next(), shape, jnp.bfloat16, lo, hi)
    def permutation(self, n):
        return jax.random.permutation(self._next(), n)


kernel_name = 'standalone__mha_softmax__near_ridge'

def _fwd_setup_inputs():
    _rng = _Rng(jax.random.key(int.from_bytes(__import__("os").urandom(4), "little")))
    _w = (lambda a: (lambda t: t.astype(jnp.bfloat16) if jnp.issubdtype(t.dtype, jnp.floating) else t)(jnp.asarray(a)))
    B, H, Sq, Sk, D = 8, 16, 512, 1024, 256
    return {
        "q": _w((lambda *s: _rng.normal(s) * 0.05)(B, H, Sq, D)),
        "k": _w((lambda *s: _rng.normal(s) * 0.05)(B, H, Sk, D)),
        "v": _w((lambda *s: _rng.normal(s) * 0.05)(B, H, Sk, D)),
    }

def _fwd_reference(q, k, v):
    scale = q.shape[-1] ** -0.5
    scores = jnp.einsum("bhqd,bhkd->bhqk", q, k) * scale
    p = _softmax(scores, axis=-1)
    return jnp.einsum("bhqk,bhkd->bhqd", p, v)


def setup_inputs():
    _inp = _fwd_setup_inputs()
    _gk = jax.random.fold_in(jax.random.key(int.from_bytes(__import__("os").urandom(4), "little")), 2**31 - 1)
    _shapes = [[8, 16, 512, 256]]
    _dtypes = ['bfloat16']
    _gks = jax.random.split(_gk, len(_shapes))
    _gs = [jax.random.normal(k, s, dtype=jnp.dtype(d)) * 0.05 for k, s, d in zip(_gks, _shapes, _dtypes)]
    _inp["grad_out"] = _gs[0]
    return _inp

def reference(q, k, v, grad_out):
    _const = dict()
    def _f(*_d):
        return _fwd_reference(**{'q': _d[0], 'k': _d[1], 'v': _d[2], **_const})
    _out, _vjp = jax.vjp(_f, q, k, v)
    _grads = _vjp(grad_out)
    _out0 = jnp.asarray(_out)
    return (_out0, *[jnp.asarray(_g) for _g in _grads])
```

```python
import functools
import jax
import jax.numpy as jnp
from jax import lax
import jax.experimental.pallas as pl
import jax.experimental.pallas.tpu as pltpu

NT = (((1,), (1,)), ((), ()))
NN = (((1,), (0,)), ((), ()))
TN = (((0,), (0,)), ((), ()))

def _kernel(q_ref, k_ref, v_ref, do_ref, o_ref, dq_ref, dk_ref, dv_ref, *, scale):
    f32 = jnp.float32
    bf = jnp.bfloat16
    q = q_ref[0]; k = k_ref[0]; v = v_ref[0]; do = do_ref[0]
    s = lax.dot_general(q, k, NT, preferred_element_type=f32) * scale
    m = jnp.max(s, axis=-1, keepdims=True)
    p = jnp.exp(s - m)
    l = jnp.sum(p, axis=-1, keepdims=True)
    inv = 1.0 / l
    pb = p.astype(bf)
    o = lax.dot_general(pb, v, NN, preferred_element_type=f32) * inv
    o_ref[0] = o.astype(bf)
    dof = do.astype(f32) * inv
    dd = jnp.sum(dof * o, axis=-1, keepdims=True)
    dob = dof.astype(bf)
    dp = lax.dot_general(dob, v, NT, preferred_element_type=f32)
    ds = (p * (dp - dd)).astype(bf)
    dv_ref[0] = lax.dot_general(pb, dob, TN, preferred_element_type=f32).astype(bf)
    dq_ref[0] = (lax.dot_general(ds, k, NN, preferred_element_type=f32) * scale).astype(bf)
    dk_ref[0] = (lax.dot_general(ds, q, TN, preferred_element_type=f32) * scale).astype(bf)


@jax.jit
def pallas_standalone__mha_softmax__near_ridge_kernel(q, k, v, grad_out):
    B, H, Sq, D = q.shape
    Sk = k.shape[2]
    BH = B * H
    q3 = q.reshape(BH, Sq, D); k3 = k.reshape(BH, Sk, D); v3 = v.reshape(BH, Sk, D)
    g3 = grad_out.reshape(BH, Sq, D)
    qspec = pl.BlockSpec((1, Sq, D), lambda i: (i, 0, 0))
    kspec = pl.BlockSpec((1, Sk, D), lambda i: (i, 0, 0))
    outs = pl.pallas_call(
        functools.partial(_kernel, scale=D ** -0.5),
        grid=(BH,),
        in_specs=[qspec, kspec, kspec, qspec],
        out_specs=[qspec, qspec, kspec, kspec],
        out_shape=[jax.ShapeDtypeStruct((BH, Sq, D), q.dtype), jax.ShapeDtypeStruct((BH, Sq, D), q.dtype),
                   jax.ShapeDtypeStruct((BH, Sk, D), q.dtype), jax.ShapeDtypeStruct((BH, Sk, D), q.dtype)],
        compiler_params=pltpu.CompilerParams(dimension_semantics=("parallel",), vmem_limit_bytes=100 * 1024 * 1024),
    )(q3, k3, v3, g3)
    o, dq, dk, dv = outs
    return (o.reshape(B, H, Sq, D), dq.reshape(B, H, Sq, D), dk.reshape(B, H, Sk, D), dv.reshape(B, H, Sk, D))
```

```python
import functools, os
import jax
import jax.numpy as jnp
from jax import lax
import jax.experimental.pallas as pl
import jax.experimental.pallas.tpu as pltpu

NT = (((1,), (1,)), ((), ()))
NN = (((1,), (0,)), ((), ()))
TN = (((0,), (0,)), ((), ()))
G = int(os.environ.get("KG", "1"))
NOBC = bool(int(os.environ.get("NOBC", "1")))
CH = [int(x) for x in os.environ.get("CH", "128,128,128,128").split(",")]
KB = int(os.environ.get("KB", "1024"))
LSEP = bool(int(os.environ.get("LSEP", "0")))
DOBP = bool(int(os.environ.get("DOBP", "1")))
DDS = bool(int(os.environ.get("DDS", "0")))
ORDER = os.environ.get("ORDER", "S0,S1,M0,S2,M1,S3,M2,O0,M3,O1,O2,O3,P0,P1,P2,P3,V,Q0,Q1,Q2,Q3,K").replace(",", " ").split()
QDL = int(os.environ.get("QDL", "-1"))
LOG2E = 1.4426950408889634
f32 = jnp.float32
bf = jnp.bfloat16
u32 = jnp.uint32
OFF = [sum(CH[:i]) for i in range(len(CH))]
NC = len(CH)

def rep(x, n):
    return jnp.concatenate([x] * n, axis=1)

class Head:
    def __init__(self, refs, scr, z0, scale):
        (self.q_ref, self.k_ref, self.v_ref, self.do_ref, self.o_ref, self.dq_ref, self.dk_ref, self.dv_ref) = refs
        self.scale = scale
        self.scr = scr; self.z0 = z0
        self.m = {}; self.dd = {}
        self.kstaged = False; self.vstaged = False
        self.Sk = self.k_ref.shape[0]; self.D = self.k_ref.shape[1]
    def dyn(self, off, n):
        return pl.ds(pl.multiple_of(off + 16 * self.z0, 16), n)
    def barrier(self, raw):
        n = raw.shape[0] - 16
        raw[self.dyn(n, 8), pl.ds(0, 128)] = jnp.zeros((8, 128), raw.dtype)
    def K(self):
        kv = self.scr["kv"][0]
        if not self.kstaged:
            self.kstaged = True
            x = self.k_ref[...]
            kv.bitcast(bf)[pl.ds(0, self.Sk), :] = x
            self.barrier(kv)
            return x
        return kv.bitcast(bf)[pl.ds(0, self.Sk), :]
    def V(self):
        kv = self.scr["kv"][1]
        if not self.vstaged:
            self.vstaged = True
            x = self.v_ref[...]
            kv.bitcast(bf)[pl.ds(0, self.Sk), :] = x
            if QDL >= 0:
                kv.bitcast(bf)[pl.ds(self.Sk, CH[QDL]), :] = self.q_ref[self.rows(QDL), :]
            self.barrier(kv)
            if "W" not in ORDER: return x
        return kv.bitcast(bf)[pl.ds(0, self.Sk), :]
    def q(self, r):
        if r == QDL:
            return self.scr["kv"][1].bitcast(bf)[pl.ds(self.Sk, CH[QDL]), :]
        return self.q_ref[self.rows(r), :]
    def rows(self, r): return pl.ds(OFF[r], CH[r])
    def p(self, r, cols=None):
        cs = slice(None) if cols is None else pl.ds(cols[0], cols[1])
        return self.scr["p"][r].bitcast(bf)[pl.ds(0, CH[r]), cs]
    def ds(self, r, cols=None):
        cs = slice(None) if cols is None else pl.ds(cols[0], cols[1])
        return self.scr["ds"][r].bitcast(bf)[pl.ds(0, CH[r]), cs]
    def inv(self, r):
        return self.scr["p"][r].bitcast(f32)[pl.ds(CH[r] // 2, CH[r]), pl.ds(0, 128)]
    def dob(self, r):
        if DOBP:
            return self.scr["p"][r].bitcast(bf)[pl.ds(CH[r], CH[r]), pl.ds(128, self.D)]
        return self.scr["dob"][r].bitcast(bf)[pl.ds(0, CH[r]), :]
    def fin(self, r, p):
        R = CH[r]
        l = jnp.sum(p, axis=-1, keepdims=True)
        inv = 1.0 / l
        raw = self.scr["p"][r]
        raw.bitcast(f32)[self.dyn(R // 2, R), pl.ds(0, 128)] = jnp.broadcast_to(inv, (R, 128))
        dob = (self.do_ref[self.rows(r), :].astype(f32) * (inv * self.scale)).astype(bf)
        if DOBP:
            raw.bitcast(bf)[self.dyn(R, R), pl.ds(128, self.D)] = dob
        else:
            d = self.scr["dob"][r]
            d.bitcast(bf)[pl.ds(0, R), :] = dob
            self.barrier(d)
    def step(self, name):
        op, arg = name[0], name[1:]
        r = int(arg) if arg else None
        scale = self.scale
        c = scale * LOG2E
        if op == "S":
            s = lax.dot_general(self.q(r), self.K(), NT, preferred_element_type=f32) * c
            self.m[r] = jnp.max(s, axis=-1, keepdims=True)
            raw = self.scr["s"][r]
            raw[pl.ds(0, CH[r]), :] = s
            self.barrier(raw)
        elif op == "W":
            self.V()
        elif op == "X":
            self.K()
        elif op == "M":
            p = jnp.exp2(self.scr["s"][r][pl.ds(0, CH[r]), :] - self.m[r])
            raw = self.scr["p"][r]
            raw.bitcast(bf)[pl.ds(0, CH[r]), :] = p.astype(bf)
            if LSEP:
                self.barrier(raw)
                self.fin(r, self.p(r).astype(f32))
            else:
                self.fin(r, p)
        elif op == "O":
            o = lax.dot_general(self.p(r), self.V(), NN, preferred_element_type=f32) * rep(self.inv(r), 2)
            self.o_ref[self.rows(r), :] = o.astype(bf)
            dd = jnp.sum(self.dob(r).astype(f32) * o, axis=-1, keepdims=True)
            if DDS:
                raw = self.scr["dd"][r]
                raw[self.dyn(0, CH[r]), :] = jnp.broadcast_to(dd, (CH[r], 128))
            else:
                self.dd[r] = dd
        elif op == "P":
            dp = lax.dot_general(self.dob(r), self.V(), NT, preferred_element_type=f32)
            p = self.p(r).astype(f32)
            raw = self.scr["ds"][r]
            dd = rep(self.scr["dd"][r][pl.ds(0, CH[r]), :], self.Sk // 128) if DDS else self.dd[r]
            raw.bitcast(bf)[pl.ds(0, CH[r]), :] = (p * (dp - dd)).astype(bf)
            self.barrier(raw)
        elif op == "V":
            dob = jnp.concatenate([self.dob(r) for r in range(NC)], axis=0)
            for j in range(0, self.Sk, KB):
                pj = jnp.concatenate([self.p(r, (j, KB)) for r in range(NC)], axis=0)
                dv = lax.dot_general(pj, dob, TN, preferred_element_type=f32) * (1.0 / scale)
                self.dv_ref[pl.ds(j, KB), :] = dv.astype(bf)
        elif op == "Q":
            self.dq_ref[self.rows(r), :] = lax.dot_general(self.ds(r), self.K(), NN, preferred_element_type=f32).astype(bf)
        elif op == "K":
            q = self.q_ref[...]
            for j in range(0, self.Sk, KB):
                dsj = jnp.concatenate([self.ds(r, (j, KB)) for r in range(NC)], axis=0)
                self.dk_ref[pl.ds(j, KB), :] = lax.dot_general(dsj, q, TN, preferred_element_type=f32).astype(bf)
        else:
            raise ValueError(name)

def _shapes(Sk, D):
    d = {}
    d["s"] = [pltpu.VMEM((c + 16, Sk), f32) for c in CH]
    d["p"] = [pltpu.VMEM((c // 2 + c + 16, Sk), u32) for c in CH]
    d["ds"] = [pltpu.VMEM((c // 2 + 16, Sk), u32) for c in CH]
    if not DOBP: d["dob"] = [pltpu.VMEM((c // 2 + 16, D), u32) for c in CH]
    if DDS: d["dd"] = [pltpu.VMEM((c + 16, 128), f32) for c in CH]
    d["kv"] = [pltpu.VMEM((Sk // 2 + 16, D), u32), pltpu.VMEM((Sk // 2 + 128 + 16, D), u32)]
    return d

def _kernel(*refs, scale, shapes):
    io = refs[:8]; scr = refs[8:]
    i = pl.program_id(0)
    z0 = (i % 2) * ((i + 1) % 2)
    heads = []
    it = iter(scr)
    for g in range(G):
        d = {n: [next(it) for _ in v] for n, v in shapes.items()}
        heads.append(Head([x.at[g] for x in io], d, z0, scale))
    if any(":" in t for t in ORDER):
        for t in ORDER:
            g, name = t.split(":")
            heads[int(g)].step(name)
    else:
        for h in heads:
            for t in ORDER:
                h.step(t)


@jax.jit
def pallas_standalone__mha_softmax__near_ridge_kernel(q, k, v, grad_out):
    B, H, Sq, D = q.shape
    Sk = k.shape[2]
    BH = B * H
    q3 = q.reshape(BH, Sq, D); k3 = k.reshape(BH, Sk, D); v3 = v.reshape(BH, Sk, D)
    g3 = grad_out.reshape(BH, Sq, D)
    qspec = pl.BlockSpec((G, Sq, D), lambda i: (i, 0, 0))
    kspec = pl.BlockSpec((G, Sk, D), lambda i: (i, 0, 0))
    shapes = _shapes(Sk, D)
    scratch = [s for g in range(G) for v in shapes.values() for s in v]
    outs = pl.pallas_call(
        functools.partial(_kernel, scale=D ** -0.5, shapes=shapes),
        grid=(BH // G,),
        in_specs=[qspec, kspec, kspec, qspec],
        out_specs=[qspec, qspec, kspec, kspec],
        out_shape=[jax.ShapeDtypeStruct((BH, Sq, D), q.dtype), jax.ShapeDtypeStruct((BH, Sq, D), q.dtype),
                   jax.ShapeDtypeStruct((BH, Sk, D), q.dtype), jax.ShapeDtypeStruct((BH, Sk, D), q.dtype)],
        scratch_shapes=scratch,
        compiler_params=pltpu.CompilerParams(dimension_semantics=("arbitrary",), vmem_limit_bytes=100 * 1024 * 1024,
                                             disable_bounds_checks=NOBC),
    )(q3, k3, v3, g3)
    o, dq, dk, dv = outs
    return (o.reshape(B, H, Sq, D), dq.reshape(B, H, Sq, D), dk.reshape(B, H, Sk, D), dv.reshape(B, H, Sk, D))
```

```python
import functools, os
import jax
import jax.numpy as jnp
from jax import lax
import jax.experimental.pallas as pl
import jax.experimental.pallas.tpu as pltpu

NT = (((1,), (1,)), ((), ()))
NN = (((1,), (0,)), ((), ()))
TN = (((0,), (0,)), ((), ()))
G = int(os.environ.get("KG", "4"))
NSET = int(os.environ.get("NSET", "4"))
NOBC = bool(int(os.environ.get("NOBC", "1")))
CH = [int(x) for x in os.environ.get("CH", "128,128,128,128").split(",")]
ORDER = os.environ.get("ORDER", "S0,S1,M0,S2,M1,S3,M2,O0,M3,O1,O2,O3,o,P0,P1,P2,P3,V,v,Q0,Q1,Q2,Q3,q,K").replace(",", " ").split()
RCP = int(os.environ.get("RCP", "2"))
KB = int(os.environ.get("KB", "256"))
PCS = int(os.environ.get("PCS", "1"))
LOG2E = 1.4426950408889634
f32 = jnp.float32
bf = jnp.bfloat16
u32 = jnp.uint32
OFF = [sum(CH[:i]) for i in range(len(CH))]
NC = len(CH)

def rep(x, n):
    return jnp.concatenate([x] * n, axis=1)

class Head:
    def __init__(self, refs, scr, z0, scale, start_out, wait_next):
        (self.q_ref, self.k_ref, self.v_ref, self.do_ref, self.o_ref, self.dq_ref, self.dk_ref, self.dv_ref) = refs
        self.scale = scale
        self.scr = scr; self.z0 = z0
        self.m = {}; self.dd = {}
        self.kstaged = False; self.vstaged = False
        self.Sk = self.k_ref.shape[0]; self.D = self.k_ref.shape[1]
        self.start_out = start_out; self.wait_next = wait_next
    def dyn(self, off, n):
        return pl.ds(pl.multiple_of(off + 16 * self.z0, 16), n)
    def barrier(self, ref):
        n = ref.shape[0] - 32
        ref[self.dyn(n, 16), pl.ds(0, 128)] = jnp.zeros((16, 128), ref.dtype)
    def stage(self, idx, src):
        ref = self.scr["kv"][idx].bitcast(bf)
        x = src[...]
        ref[pl.ds(0, self.Sk), :] = x
        self.barrier(ref)
        return x
    def K(self):
        if not self.kstaged:
            self.kstaged = True
            return self.stage(0, self.k_ref)
        return self.scr["kv"][0].bitcast(bf)[pl.ds(0, self.Sk), :]
    def V(self):
        if not self.vstaged:
            self.vstaged = True
            return self.stage(1, self.v_ref)
        return self.scr["kv"][1].bitcast(bf)[pl.ds(0, self.Sk), :]
    def rows(self, r): return pl.ds(OFF[r], CH[r])
    def p(self, r): return self.scr["p"][r].bitcast(bf)[pl.ds(0, CH[r]), :]
    def ds(self, r): return self.scr["ds"][r].bitcast(bf)[pl.ds(0, CH[r]), :]
    def inv(self, r): return self.scr["inv"][r][pl.ds(0, CH[r]), :]
    def dob(self, r): return self.scr["p"][r].bitcast(bf)[pl.ds(CH[r], CH[r]), pl.ds(0, self.D)]
    def step(self, name):
        op, arg = name[0], name[1:]
        r = int(arg) if arg else None
        scale = self.scale
        c = scale * LOG2E
        if op == "S":
            s = lax.dot_general(self.q_ref[self.rows(r), :], self.K(), NT, preferred_element_type=f32) * c
            self.m[r] = jnp.max(s, axis=-1, keepdims=True)
            ref = self.scr["s"][r]
            ref[pl.ds(0, CH[r]), :] = s
            self.barrier(ref)
        elif op == "M":
            R = CH[r]
            p = jnp.exp2(self.scr["s"][r][pl.ds(0, R), :] - self.m[r])
            ref = self.scr["p"][r].bitcast(bf)
            ref[pl.ds(0, R), :] = p.astype(bf)
            l = jnp.sum(p, axis=-1, keepdims=True)
            if RCP == 0:
                inv = 1.0 / l
            elif RCP == 1:
                r0 = pl.reciprocal(l, approx=True)
                inv = r0 * (2.0 - l * r0)
            else:
                inv = pl.reciprocal(l, approx=True)
            self.scr["inv"][r][self.dyn(0, R), :] = jnp.broadcast_to(inv, (R, 128))
            dob = (self.do_ref[self.rows(r), :].astype(f32) * (inv * scale)).astype(bf)
            ref[self.dyn(R, R), pl.ds(0, self.D)] = dob
        elif op == "O":
            o = lax.dot_general(self.p(r), self.V(), NN, preferred_element_type=f32) * rep(self.inv(r), self.D // 128)
            self.o_ref[self.rows(r), :] = o.astype(bf)
            self.dd[r] = jnp.sum(self.dob(r).astype(f32) * o, axis=-1, keepdims=True)
        elif op == "P":
            dp = lax.dot_general(self.dob(r), self.V(), NT, preferred_element_type=f32)
            p = self.p(r).astype(f32)
            ref = self.scr["ds"][r].bitcast(bf)
            ref[pl.ds(0, CH[r]), :] = (p * (dp - self.dd[r])).astype(bf)
            self.barrier(ref)
        elif op == "V":
            dob = jnp.concatenate([self.dob(r) for r in range(NC)], axis=0)
            p = jnp.concatenate([self.p(r) for r in range(NC)], axis=0)
            dv = lax.dot_general(p, dob, TN, preferred_element_type=f32) * (1.0 / scale)
            self.dv_ref[...] = dv.astype(bf)
        elif op == "Q":
            self.dq_ref[self.rows(r), :] = lax.dot_general(self.ds(r), self.K(), NN, preferred_element_type=f32).astype(bf)
        elif op == "K":
            ds = jnp.concatenate([self.ds(r) for r in range(NC)], axis=0)
            dk = lax.dot_general(ds, self.q_ref[...], TN, preferred_element_type=f32)
            for j in range(0, self.Sk, KB):
                self.dk_ref[pl.ds(j, KB), :] = dk[j:j + KB].astype(bf)
                self.start_out(2, j, KB)
        elif op in "oqv":
            self.start_out({"o": 0, "q": 1, "v": 3}[op])
        elif op == "N":
            self.wait_next()
        else:
            raise ValueError(name)

def _shapes(Sk, D):
    d = {}
    d["s"] = [pltpu.VMEM((c + 32, Sk), f32) for c in CH]
    d["p"] = [pltpu.VMEM((c + 16, Sk), u32) for c in CH]
    d["ds"] = [pltpu.VMEM((c // 2 + 16, Sk), u32) for c in CH]
    d["inv"] = [pltpu.VMEM((c + 16, 128), f32) for c in CH]
    d["kv"] = [pltpu.VMEM((Sk // 2 + 16, D), u32), pltpu.VMEM((Sk // 2 + 16, D), u32)]
    return d

def _kernel(*refs, scale, shapes, nsteps, Sq, Sk):
    hbm_in = refs[:4]; hbm_out = refs[4:8]
    buf_in, buf_out, sem_a, sem_in, sem_out, z_ref = refs[8:14]
    scr = refs[14:]
    sizes_in = (Sq, Sk, Sk, Sq)
    sizes_out = (Sq, Sq, Sk, Sk)
    off_in = [sum(sizes_in[:a]) for a in range(4)]
    off_out = [sum(sizes_out[:a]) for a in range(4)]
    in_order = (1, 0, 3, 2)

    def start_in(step, sl):
        for a in in_order:
            pltpu.make_async_copy(hbm_in[a].at[pl.ds(step * G, G)],
                                  buf_in.at[sl, :, pl.ds(off_in[a], sizes_in[a]), :], sem_in.at[sl]).start()
    def wait_in(sl):
        pltpu.make_async_copy(buf_in.at[sl], buf_in.at[sl], sem_in.at[sl]).wait()
    def start_head(g, pieces=1):
        for a in in_order:
            n = sizes_in[a] // pieces
            for j in range(pieces):
                pltpu.make_async_copy(hbm_in[a].at[g, pl.ds(j * n, n), :],
                                      buf_in.at[0, g, pl.ds(off_in[a] + j * n, n), :], sem_a.at[g]).start()
    def wait_head(g):
        pltpu.make_async_copy(buf_in.at[0, g], buf_in.at[0, g], sem_a.at[g]).wait()
    def start_out(step, sl, g, a, r0=0, n=None):
        n = sizes_out[a] if n is None else n
        pltpu.make_async_copy(buf_out.at[sl, g, pl.ds(off_out[a] + r0, n), :],
                              hbm_out[a].at[step * G + g, pl.ds(r0, n), :], sem_out.at[sl]).start()
    def wait_out(sl):
        pltpu.make_async_copy(buf_out.at[sl], buf_out.at[sl], sem_out.at[sl]).wait()

    sets = []
    it = iter(scr)
    for _ in range(NSET):
        sets.append({n: [next(it) for _ in v] for n, v in shapes.items()})

    def run_head(step, slot, g, z0, scr_set):
        io = ([buf_in.at[slot, g, pl.ds(off_in[a], sizes_in[a]), :] for a in range(4)]
              + [buf_out.at[slot, g, pl.ds(off_out[a], sizes_out[a]), :] for a in range(4)])
        h = Head(io, scr_set, z0, scale, start_out=lambda *a: start_out(step, slot, g, *a), wait_next=lambda: None)
        for t in ORDER:
            h.step(t)

    z_ref[0] = 0
    start_head(0, PCS)
    wait_head(0)
    for g in range(1, G):
        start_head(g)

    def body_a(g, carry):
        z0 = z_ref[0]
        @pl.when(g == 1)
        def _():
            start_in(1, 1)
        @pl.when(g >= 1)
        def _():
            wait_head(g)
        run_head(0, 0, g, z0, sets[0])
        return carry

    def body(i, carry):
        slot = i & 1

        @pl.when(i == 0)
        def _():
            lax.fori_loop(0, G, body_a, 0)
            start_in(2, 0)
            wait_in(1)

        @pl.when(i > 0)
        def _():
            z0 = z_ref[0]
            for g in range(G):
                run_head(i, slot, g, z0, sets[g % NSET])

            @pl.when(i + 2 < nsteps)
            def _():
                start_in(i + 2, slot)

            @pl.when(i + 1 < nsteps)
            def _():
                wait_in(1 - slot)
            wait_out(1 - slot)
        return carry

    lax.fori_loop(0, nsteps, body, 0)
    wait_out((nsteps - 1) % 2)


@jax.jit
def pallas_standalone__mha_softmax__near_ridge_kernel(q, k, v, grad_out):
    B, H, Sq, D = q.shape
    Sk = k.shape[2]
    BH = B * H
    q2 = q.reshape(BH, Sq, D); k2 = k.reshape(BH, Sk, D); v2 = v.reshape(BH, Sk, D)
    g2 = grad_out.reshape(BH, Sq, D)
    shapes = _shapes(Sk, D)
    nsteps = int(os.environ.get("NH", BH)) // G
    rows = 2 * (Sq + Sk)
    scratch = [pltpu.VMEM((2, G, rows, D), bf), pltpu.VMEM((2, G, rows, D), bf),
               pltpu.SemaphoreType.DMA((G,)), pltpu.SemaphoreType.DMA((2,)), pltpu.SemaphoreType.DMA((2,)),
               pltpu.SMEM((1,), jnp.int32)]
    scratch += [s for _ in range(NSET) for v in shapes.values() for s in v]
    anyspec = pl.BlockSpec(memory_space=pl.ANY)
    outs = pl.pallas_call(
        functools.partial(_kernel, scale=D ** -0.5, shapes=shapes, nsteps=nsteps, Sq=Sq, Sk=Sk),
        in_specs=[anyspec] * 4,
        out_specs=[anyspec] * 4,
        out_shape=[jax.ShapeDtypeStruct((BH, Sq, D), q.dtype), jax.ShapeDtypeStruct((BH, Sq, D), q.dtype),
                   jax.ShapeDtypeStruct((BH, Sk, D), q.dtype), jax.ShapeDtypeStruct((BH, Sk, D), q.dtype)],
        scratch_shapes=scratch,
        compiler_params=pltpu.CompilerParams(vmem_limit_bytes=110 * 1024 * 1024,
                                             disable_bounds_checks=NOBC),
    )(q2, k2, v2, g2)
    o, dq, dk, dv = outs
    return (o.reshape(B, H, Sq, D), dq.reshape(B, H, Sq, D), dk.reshape(B, H, Sk, D), dv.reshape(B, H, Sk, D))
```

```python
import functools

import jax
import jax.numpy as jnp
from jax import lax
import jax.experimental.pallas as pl
import jax.experimental.pallas.tpu as pltpu

_NT = (((1,), (1,)), ((), ()))
_NN = (((1,), (0,)), ((), ()))
_TN = (((0,), (0,)), ((), ()))
_LOG2E = 1.4426950408889634
_F32 = jnp.float32
_BF16 = jnp.bfloat16
_U32 = jnp.uint32

_G = 4
_NSET = 2
_R = 128
_KB = 256
_PAD = 16


def _pack(x):
    return pltpu.bitcast(x, _U32)


def _unpack(x):
    return pltpu.bitcast(x, _BF16)


def _dot(a, b, dims):
    return lax.dot_general(a, b, dims, preferred_element_type=_F32)


def _one_head(q_ref, k_ref, v_ref, do_ref, o_ref, dq_ref, dk_ref, dv_ref,
              scr, zero, scale, start_out):
    sq, d = q_ref.shape
    sk = k_ref.shape[0]
    nc = sq // _R
    s_scr, p_scr, ds_scr, inv_scr, (k_scr, v_scr) = scr

    def fence(ref):
        n = ref.shape[0] - _PAD
        ref[pl.ds(pl.multiple_of(n + 8 * zero, 8), 8), pl.ds(0, 128)] = jnp.zeros((8, 128), ref.dtype)

    def staged(src, dst):
        state = {"done": False}

        def get():
            if state["done"]:
                return _unpack(dst[pl.ds(0, sk // 2), :])
            state["done"] = True
            x = src[...]
            dst[pl.ds(0, sk // 2), :] = _pack(x)
            fence(dst)
            return x
        return get

    get_k = staged(k_ref, k_scr)
    get_v = staged(v_ref, v_scr)
    rows = lambda r: pl.ds(r * _R, _R)
    get_p = lambda r: _unpack(p_scr[r][pl.ds(0, _R // 2), :])
    get_dob = lambda r: _unpack(p_scr[r][pl.ds(_R // 2, _R // 2), pl.ds(0, d)])
    get_ds = lambda r: _unpack(ds_scr[r][pl.ds(0, _R // 2), :])
    row_max = {}
    delta = {}

    def scores(r):
        s = _dot(q_ref[rows(r), :], get_k(), _NT) * (scale * _LOG2E)
        row_max[r] = jnp.max(s, axis=-1, keepdims=True)
        s_scr[r][pl.ds(0, _R), :] = s
        fence(s_scr[r])

    def softmax(r):
        p = jnp.exp2(s_scr[r][pl.ds(0, _R), :] - row_max[r])
        p_scr[r][pl.ds(0, _R // 2), :] = _pack(p.astype(_BF16))
        inv = pl.reciprocal(jnp.sum(p, axis=-1, keepdims=True), approx=True)
        inv_scr[r][pl.ds(0, _R), :] = jnp.broadcast_to(inv, (_R, 128))
        fence(inv_scr[r])
        dob = (do_ref[rows(r), :].astype(_F32) * (inv * scale)).astype(_BF16)
        p_scr[r][pl.ds(_R // 2, _R // 2), pl.ds(0, d)] = _pack(dob)
        fence(p_scr[r])

    def out(r):
        inv = inv_scr[r][pl.ds(0, _R), :]
        o = _dot(get_p(r), get_v(), _NN) * jnp.concatenate([inv] * (d // 128), axis=1)
        o_ref[rows(r), :] = o.astype(_BF16)
        delta[r] = jnp.sum(get_dob(r).astype(_F32) * o, axis=-1, keepdims=True)

    def dscores(r):
        dp = _dot(get_dob(r), get_v(), _NT)
        ds = get_p(r).astype(_F32) * (dp - delta[r])
        ds_scr[r][pl.ds(0, _R // 2), :] = _pack(ds.astype(_BF16))
        fence(ds_scr[r])

    scores(0)
    for r in range(1, nc):
        scores(r)
        softmax(r - 1)
    out(0)
    softmax(nc - 1)
    for r in range(1, nc):
        out(r)
    start_out(0, 0, sq)
    for r in range(nc):
        dscores(r)
    for r in range(nc):
        dq_ref[rows(r), :] = _dot(get_ds(r), get_k(), _NN).astype(_BF16)
    start_out(1, 0, sq)

    dob = jnp.concatenate([get_dob(r) for r in range(nc)], axis=0)
    p = jnp.concatenate([get_p(r) for r in range(nc)], axis=0)
    dv_ref[...] = (_dot(p, dob, _TN) * (1.0 / scale)).astype(_BF16)
    start_out(3, 0, sk)

    ds = jnp.concatenate([get_ds(r) for r in range(nc)], axis=0)
    dk = _dot(ds, q_ref[...], _TN)
    for j in range(0, sk, _KB):
        dk_ref[pl.ds(j, _KB), :] = dk[j:j + _KB].astype(_BF16)
        start_out(2, j, _KB)


def _scratch_set(sq, sk, d):
    nc = sq // _R
    return ([pltpu.VMEM((_R + _PAD, sk), _F32) for _ in range(nc)]
            + [pltpu.VMEM((_R + _PAD, sk), _U32) for _ in range(nc)]
            + [pltpu.VMEM((_R // 2 + _PAD, sk), _U32) for _ in range(nc)]
            + [pltpu.VMEM((_R + _PAD, 128), _F32) for _ in range(nc)]
            + [pltpu.VMEM((sk // 2 + _PAD, d), _U32) for _ in range(2)])


def _kernel(q_hbm, k_hbm, v_hbm, do_hbm, o_hbm, dq_hbm, dk_hbm, dv_hbm,
            buf_in, buf_out, sem_head, sem_in, sem_out, zero_ref, *scr, scale):
    hbm_in = (q_hbm, k_hbm, v_hbm, do_hbm)
    hbm_out = (o_hbm, dq_hbm, dk_hbm, dv_hbm)
    nblk = q_hbm.shape[0] // _G
    sq, sk = q_hbm.shape[1], k_hbm.shape[1]
    nc = sq // _R
    len_in = (sq, sk, sk, sq)
    len_out = (sq, sq, sk, sk)
    off_in = [sum(len_in[:a]) for a in range(4)]
    off_out = [sum(len_out[:a]) for a in range(4)]
    in_order = (1, 0, 3, 2)

    per_set = len(scr) // _NSET
    sets = []
    for t in range(_NSET):
        s = scr[t * per_set:(t + 1) * per_set]
        sets.append((s[0:nc], s[nc:2 * nc], s[2 * nc:3 * nc], s[3 * nc:4 * nc], s[4 * nc:]))

    def start_block(blk, slot):
        for a in in_order:
            pltpu.make_async_copy(hbm_in[a].at[pl.ds(blk * _G, _G)],
                                  buf_in.at[slot, :, pl.ds(off_in[a], len_in[a]), :],
                                  sem_in.at[slot]).start()

    def wait_block(slot):
        pltpu.make_async_copy(buf_in.at[slot], buf_in.at[slot], sem_in.at[slot]).wait()

    def start_head(g):
        for a in in_order:
            pltpu.make_async_copy(hbm_in[a].at[g],
                                  buf_in.at[0, g, pl.ds(off_in[a], len_in[a]), :],
                                  sem_head.at[g]).start()

    def wait_head(g):
        pltpu.make_async_copy(buf_in.at[0, g], buf_in.at[0, g], sem_head.at[g]).wait()

    def wait_out(blk, slot):
        for a in range(4):
            pltpu.make_async_copy(buf_out.at[slot, :, pl.ds(off_out[a], len_out[a]), :],
                                  hbm_out[a].at[pl.ds(blk * _G, _G)],
                                  sem_out.at[slot * 4 + a]).wait()

    def run_head(blk, slot, g, zero, scr_set):
        def start_out(a, r0, n):
            pltpu.make_async_copy(buf_out.at[slot, g, pl.ds(off_out[a] + r0, n), :],
                                  hbm_out[a].at[blk * _G + g, pl.ds(r0, n), :],
                                  sem_out.at[slot * 4 + a]).start()
        ins = [buf_in.at[slot, g, pl.ds(off_in[a], len_in[a]), :] for a in range(4)]
        outs = [buf_out.at[slot, g, pl.ds(off_out[a], len_out[a]), :] for a in range(4)]
        _one_head(*ins, *outs, scr_set, zero, scale, start_out)

    zero_ref[0] = 0

    start_head(0)
    wait_head(0)
    for g in range(1, _G):
        start_head(g)

    def first_block(g, carry):
        @pl.when(g == 1)
        def _():
            start_block(1, 1)

        @pl.when(g >= 1)
        def _():
            wait_head(g)

        run_head(0, 0, g, zero_ref[0], sets[0])
        return carry

    lax.fori_loop(0, _G, first_block, 0)
    start_block(2, 0)
    wait_block(1)

    def block(i, carry):
        slot = i & 1
        zero = zero_ref[0]
        for g in range(_G):
            run_head(i, slot, g, zero, sets[g % _NSET])

        @pl.when(i + 2 < nblk)
        def _():
            start_block(i + 2, slot)

        @pl.when(i + 1 < nblk)
        def _():
            wait_block(1 - slot)

        wait_out(i - 1, 1 - slot)
        return carry

    lax.fori_loop(1, nblk, block, 0)
    wait_out(nblk - 1, (nblk - 1) % 2)


@jax.jit
def pallas_standalone__mha_softmax__near_ridge_kernel(
    q: jax.Array,
    k: jax.Array,
    v: jax.Array,
    grad_out: jax.Array,
):
    b, h, sq, d = q.shape
    sk = k.shape[2]
    bh = b * h
    assert bh % _G == 0 and bh // _G >= 3 and sq % _R == 0 and sk % _KB == 0 and d % 128 == 0
    rows = 2 * (sq + sk)
    scratch = [
        pltpu.VMEM((2, _G, rows, d), _BF16),
        pltpu.VMEM((2, _G, rows, d), _BF16),
        pltpu.SemaphoreType.DMA((_G,)),
        pltpu.SemaphoreType.DMA((2,)),
        pltpu.SemaphoreType.DMA((8,)),
        pltpu.SMEM((1,), jnp.int32),
    ]
    for _ in range(_NSET):
        scratch += _scratch_set(sq, sk, d)
    any_spec = pl.BlockSpec(memory_space=pl.ANY)
    q_shape = jax.ShapeDtypeStruct((bh, sq, d), q.dtype)
    k_shape = jax.ShapeDtypeStruct((bh, sk, d), q.dtype)
    o, dq, dk, dv = pl.pallas_call(
        functools.partial(_kernel, scale=d ** -0.5),
        in_specs=[any_spec] * 4,
        out_specs=[any_spec] * 4,
        out_shape=[q_shape, q_shape, k_shape, k_shape],
        scratch_shapes=scratch,
        compiler_params=pltpu.CompilerParams(
            vmem_limit_bytes=100 * 1024 * 1024,
            disable_bounds_checks=True,
        ),
    )(q.reshape(bh, sq, d), k.reshape(bh, sk, d), v.reshape(bh, sk, d),
      grad_out.reshape(bh, sq, d))
    return (o.reshape(b, h, sq, d), dq.reshape(b, h, sq, d),
            dk.reshape(b, h, sk, d), dv.reshape(b, h, sk, d))
```

```python
import functools

import jax
import jax.numpy as jnp
from jax import lax
import jax.experimental.pallas as pl
import jax.experimental.pallas.tpu as pltpu

_NT = (((1,), (1,)), ((), ()))
_NN = (((1,), (0,)), ((), ()))
_TN = (((0,), (0,)), ((), ()))
_LOG2E = 1.4426950408889634
_F32 = jnp.float32
_BF16 = jnp.bfloat16
_U32 = jnp.uint32

_G = 4
_NSET = 2
_R = 128
_KB = 128
_KT = 256
_PAD = 16


def _pack(x):
    return pltpu.bitcast(x, _U32)


def _unpack(x):
    return pltpu.bitcast(x, _BF16)


def _dot(a, b, dims):
    return lax.dot_general(a, b, dims, preferred_element_type=_F32)


def _one_head(q_ref, k_ref, v_ref, do_ref, o_ref, dq_ref, dk_ref, dv_ref,
              scr, zero, scale, start_out, kt_ref=None):
    sq, d = q_ref.shape
    sk = k_ref.shape[0]
    nc = sq // _R
    s_scr, p_scr, ds_scr, inv_scr, (k_scr, v_scr) = scr

    def fence(ref):
        n = ref.shape[0] - _PAD
        ref[pl.ds(pl.multiple_of(n + 8 * zero, 8), 8), pl.ds(0, 128)] = jnp.zeros((8, 128), ref.dtype)

    def staged(src, dst):
        state = {"done": False}

        def get():
            if state["done"]:
                return _unpack(dst[pl.ds(0, sk // 2), :])
            state["done"] = True
            x = src[...]
            dst[pl.ds(0, sk // 2), :] = _pack(x)
            fence(dst)
            return x
        return get

    get_k = staged(k_ref, k_scr)
    get_v = staged(v_ref, v_scr)
    rows = lambda r: pl.ds(r * _R, _R)
    get_p = lambda r: _unpack(p_scr[r][pl.ds(0, _R // 2), :])
    get_dob = lambda r: _unpack(p_scr[r][pl.ds(_R // 2, _R // 2), pl.ds(0, d)])
    get_ds = lambda r: _unpack(ds_scr[r][pl.ds(0, _R // 2), :])
    row_max = {}
    delta = {}

    def scores(r):
        if r == 0 and kt_ref is not None:
            q0 = q_ref[rows(0), :]
            s_lo = _dot(q0, _unpack(kt_ref[...]), _NN)
            s = jnp.concatenate([s_lo, _dot(q0, get_k()[_KT:], _NT)], axis=1) * (scale * _LOG2E)
        else:
            s = _dot(q_ref[rows(r), :], get_k(), _NT) * (scale * _LOG2E)
        row_max[r] = jnp.max(s, axis=-1, keepdims=True)
        s_scr[r][pl.ds(0, _R), :] = s
        fence(s_scr[r])

    def softmax(r):
        p = jnp.exp2(s_scr[r][pl.ds(0, _R), :] - row_max[r])
        p_scr[r][pl.ds(0, _R // 2), :] = _pack(p.astype(_BF16))
        inv = pl.reciprocal(jnp.sum(p, axis=-1, keepdims=True), approx=True)
        inv_scr[r][pl.ds(0, _R), :] = jnp.broadcast_to(inv, (_R, 128))
        fence(inv_scr[r])
        dob = (do_ref[rows(r), :].astype(_F32) * (inv * scale)).astype(_BF16)
        p_scr[r][pl.ds(_R // 2, _R // 2), pl.ds(0, d)] = _pack(dob)
        fence(p_scr[r])

    def out(r):
        inv = inv_scr[r][pl.ds(0, _R), :]
        o = _dot(get_p(r), get_v(), _NN) * jnp.concatenate([inv] * (d // 128), axis=1)
        o_ref[rows(r), :] = o.astype(_BF16)
        delta[r] = jnp.sum(get_dob(r).astype(_F32) * o, axis=-1, keepdims=True)

    def dscores(r):
        dp = _dot(get_dob(r), get_v(), _NT)
        ds = get_p(r).astype(_F32) * (dp - delta[r])
        ds_scr[r][pl.ds(0, _R // 2), :] = _pack(ds.astype(_BF16))
        fence(ds_scr[r])

    scores(0)
    for r in range(1, nc):
        scores(r)
        softmax(r - 1)
    out(0)
    softmax(nc - 1)
    for r in range(1, nc):
        out(r)
    start_out(0, 0, sq)
    for r in range(nc):
        dscores(r)
    for r in range(nc):
        dq_ref[rows(r), :] = _dot(get_ds(r), get_k(), _NN).astype(_BF16)
    start_out(1, 0, sq)

    dob = jnp.concatenate([get_dob(r) for r in range(nc)], axis=0)
    p = jnp.concatenate([get_p(r) for r in range(nc)], axis=0)
    dv_ref[...] = (_dot(p, dob, _TN) * (1.0 / scale)).astype(_BF16)
    start_out(3, 0, sk)

    ds = jnp.concatenate([get_ds(r) for r in range(nc)], axis=0)
    dk = _dot(ds, q_ref[...], _TN)
    for j in range(0, sk, _KB):
        dk_ref[pl.ds(j, _KB), :] = dk[j:j + _KB].astype(_BF16)
        start_out(2, j, _KB)


def _scratch_set(sq, sk, d):
    nc = sq // _R
    return ([pltpu.VMEM((_R + _PAD, sk), _F32) for _ in range(nc)]
            + [pltpu.VMEM((_R + _PAD, sk), _U32) for _ in range(nc)]
            + [pltpu.VMEM((_R // 2 + _PAD, sk), _U32) for _ in range(nc)]
            + [pltpu.VMEM((_R + _PAD, 128), _F32) for _ in range(nc)]
            + [pltpu.VMEM((sk // 2 + _PAD, d), _U32) for _ in range(2)])


def _kernel(q_hbm, k_hbm, v_hbm, do_hbm, o_hbm, dq_hbm, dk_hbm, dv_hbm,
            buf_in, buf_out, sem_head, sem_in, sem_out, zero_ref, kpre, kt_scr, sem_k, *scr, scale):
    hbm_in = (q_hbm, k_hbm, v_hbm, do_hbm)
    hbm_out = (o_hbm, dq_hbm, dk_hbm, dv_hbm)
    nblk = q_hbm.shape[0] // _G
    sq, sk = q_hbm.shape[1], k_hbm.shape[1]
    nc = sq // _R
    len_in = (sq, sk, sk, sq)
    len_out = (sq, sq, sk, sk)
    off_in = [sum(len_in[:a]) for a in range(4)]
    off_out = [sum(len_out[:a]) for a in range(4)]
    in_order = (1, 0, 3, 2)

    per_set = len(scr) // _NSET
    sets = []
    for t in range(_NSET):
        s = scr[t * per_set:(t + 1) * per_set]
        sets.append((s[0:nc], s[nc:2 * nc], s[2 * nc:3 * nc], s[3 * nc:4 * nc], s[4 * nc:]))

    def start_block(blk, slot):
        for a in in_order:
            pltpu.make_async_copy(hbm_in[a].at[pl.ds(blk * _G, _G)],
                                  buf_in.at[slot, :, pl.ds(off_in[a], len_in[a]), :],
                                  sem_in.at[slot]).start()

    def wait_block(slot):
        pltpu.make_async_copy(buf_in.at[slot], buf_in.at[slot], sem_in.at[slot]).wait()

    def start_head(g):
        for a in in_order:
            pltpu.make_async_copy(hbm_in[a].at[g],
                                  buf_in.at[0, g, pl.ds(off_in[a], len_in[a]), :],
                                  sem_head.at[g]).start()

    def wait_head(g):
        pltpu.make_async_copy(buf_in.at[0, g], buf_in.at[0, g], sem_head.at[g]).wait()

    def wait_out(blk, slot):
        for a in range(4):
            pltpu.make_async_copy(buf_out.at[slot, :, pl.ds(off_out[a], len_out[a]), :],
                                  hbm_out[a].at[pl.ds(blk * _G, _G)],
                                  sem_out.at[slot * 4 + a]).wait()

    def kpre_copy(blk, slot):
        return pltpu.make_async_copy(k_hbm.at[blk * _G, pl.ds(0, _KT), :], kpre.at[slot], sem_k.at[slot])

    def make_kt(slot):
        kt_scr[...] = _pack(kpre[slot].T)

    def run_head(blk, slot, g, zero, scr_set, kt_ref=None):
        def start_out(a, r0, n):
            pltpu.make_async_copy(buf_out.at[slot, g, pl.ds(off_out[a] + r0, n), :],
                                  hbm_out[a].at[blk * _G + g, pl.ds(r0, n), :],
                                  sem_out.at[slot * 4 + a]).start()
        ins = [buf_in.at[slot, g, pl.ds(off_in[a], len_in[a]), :] for a in range(4)]
        outs = [buf_out.at[slot, g, pl.ds(off_out[a], len_out[a]), :] for a in range(4)]
        _one_head(*ins, *outs, scr_set, zero, scale, start_out, kt_ref)

    zero_ref[0] = 0

    start_head(0)
    wait_head(0)
    for g in range(1, _G):
        start_head(g)
    kpre_copy(2, 0).start()
    kpre_copy(3, 1).start()

    def first_block(g, carry):
        @pl.when(g == 1)
        def _():
            start_block(1, 1)

        @pl.when(g >= 1)
        def _():
            wait_head(g)

        @pl.when(g == _G - 1)
        def _():
            wait_block(1)

        run_head(0, 0, g, zero_ref[0], sets[0])
        src = (g == _G - 1).astype(jnp.int32)
        kt_scr[...] = _pack(buf_in[src, 0, pl.ds(off_in[1], _KT), :].T)
        return carry

    lax.fori_loop(0, _G, first_block, 0)
    start_block(2, 0)
    kpre_copy(2, 0).wait()

    def block(i, carry):
        slot = i & 1
        zero = zero_ref[0]
        for g in range(_G):
            run_head(i, slot, g, zero, sets[g % _NSET], kt_scr if g == 0 else None)
        make_kt(1 - slot)

        @pl.when(i + 3 < nblk)
        def _():
            kpre_copy(i + 3, 1 - slot).start()

        @pl.when(i + 2 < nblk)
        def _():
            start_block(i + 2, slot)
            kpre_copy(i + 2, slot).wait()

        @pl.when(i + 1 < nblk)
        def _():
            wait_block(1 - slot)

        wait_out(i - 1, 1 - slot)
        return carry

    lax.fori_loop(1, nblk, block, 0)
    wait_out(nblk - 1, (nblk - 1) % 2)


@jax.jit
def pallas_standalone__mha_softmax__near_ridge_kernel(
    q: jax.Array,
    k: jax.Array,
    v: jax.Array,
    grad_out: jax.Array,
):
    b, h, sq, d = q.shape
    sk = k.shape[2]
    bh = b * h
    assert bh % _G == 0 and bh // _G >= 4 and sq % _R == 0 and d % 128 == 0
    assert sk % _KB == 0 and sk > _KT and sk >= d
    rows = 2 * (sq + sk)
    scratch = [
        pltpu.VMEM((2, _G, rows, d), _BF16),
        pltpu.VMEM((2, _G, rows, d), _BF16),
        pltpu.SemaphoreType.DMA((_G,)),
        pltpu.SemaphoreType.DMA((2,)),
        pltpu.SemaphoreType.DMA((8,)),
        pltpu.SMEM((1,), jnp.int32),
        pltpu.VMEM((2, _KT, d), _BF16),
        pltpu.VMEM((d // 2, _KT), _U32),
        pltpu.SemaphoreType.DMA((2,)),
    ]
    for _ in range(_NSET):
        scratch += _scratch_set(sq, sk, d)
    any_spec = pl.BlockSpec(memory_space=pl.ANY)
    q_shape = jax.ShapeDtypeStruct((bh, sq, d), q.dtype)
    k_shape = jax.ShapeDtypeStruct((bh, sk, d), q.dtype)
    o, dq, dk, dv = pl.pallas_call(
        functools.partial(_kernel, scale=d ** -0.5),
        in_specs=[any_spec] * 4,
        out_specs=[any_spec] * 4,
        out_shape=[q_shape, q_shape, k_shape, k_shape],
        scratch_shapes=scratch,
        compiler_params=pltpu.CompilerParams(
            vmem_limit_bytes=100 * 1024 * 1024,
            disable_bounds_checks=True,
        ),
    )(q.reshape(bh, sq, d), k.reshape(bh, sk, d), v.reshape(bh, sk, d),
      grad_out.reshape(bh, sq, d))
    return (o.reshape(b, h, sq, d), dq.reshape(b, h, sq, d),
            dk.reshape(b, h, sk, d), dv.reshape(b, h, sk, d))
```
